```python
import os as _os
_os.environ.setdefault("JAX_PLATFORMS", "cpu")
import jax
import jax.numpy as jnp

def _softmax(x, axis=-1):
    return jax.nn.softmax(x, axis=axis)
def _gelu(x):
    return jax.nn.gelu(x, approximate=True)
def _silu(x):
    return jax.nn.silu(x)
def _sigmoid(x):
    return jax.nn.sigmoid(x)
def _layernorm(x, axis=-1, eps=1e-5):
    m = jnp.mean(x, axis=axis, keepdims=True)
    v = jnp.var(x, axis=axis, keepdims=True)
    return (x - m) / jnp.sqrt(v + eps)
def _scatter_add(tgt, idx, src, axis=0):
    return tgt.at[idx].add(src)
def _segment_sum(src, seg, n):
    return jax.ops.segment_sum(src, seg, n)
class _Rng:
    def __init__(self, key):
        self._k = key
    def _next(self):
        self._k, sub = jax.random.split(self._k)
        return sub
    def normal(self, shape):
        return jax.random.normal(self._next(), shape, dtype=jnp.bfloat16)
    def randint(self, lo, hi, shape):
        return jax.random.randint(self._next(), shape, lo, hi, dtype=jnp.int32)
    def uniform(self, shape, lo=0.0, hi=1.0):
        return jax.random.uniform(self._next(), shape, jnp.bfloat16, lo, hi)
    def permutation(self, n):
        return jax.random.permutation(self._next(), n)


kernel_name = 'sequential_preLN__mha_block__moe_arch_mod__prompt'

def setup_inputs():
    _rng = _Rng(jax.random.key(int.from_bytes(__import__("os").urandom(4), "little")))
    _w = (lambda a: (lambda t: t.astype(jnp.bfloat16) if jnp.issubdtype(t.dtype, jnp.floating) else t)(jnp.asarray(a)))
    def _A_setup():
        B, S, D, H = 1, 2048, 512, 32
        return {
            "x": _w((lambda *s: _rng.normal(s) * 0.05)(B, S, D)),
            "wqkv": _w((lambda *s: _rng.normal(s) * 0.05)(D, 3 * D)),
            "wo": _w((lambda *s: _rng.normal(s) * 0.05)(D, D)),
        }
    _A_in = _A_setup()

    def _B_setup():
        B, S, D, F, C = 1, 2048, 512, 1792, 2
        return {
            "x": _w((lambda *s: _rng.normal(s) * 0.05)(B, S, D)),
            "w_r": _w((lambda *s: _rng.normal(s) * 0.05)(D)),
            "w_gate": _w((lambda *s: _rng.normal(s) * 0.05)(D, F)),
            "w_up": _w((lambda *s: _rng.normal(s) * 0.05)(D, F)),
            "w_down": _w((lambda *s: _rng.normal(s) * 0.05)(F, D)),
        }
    _B_in = _B_setup()

    return {
        "A_x": _A_in["x"],
        "A_wqkv": _A_in["wqkv"],
        "A_wo": _A_in["wo"],
        "B_x": _B_in["x"],
        "B_w_r": _B_in["w_r"],
        "B_w_gate": _B_in["w_gate"],
        "B_w_up": _B_in["w_up"],
        "B_w_down": _B_in["w_down"],
    }

def reference(A_x, A_wqkv, A_wo, B_x, B_w_r, B_w_gate, B_w_up, B_w_down):
    def _A_ref(x, wqkv, wo):
        B, S, D = x.shape
        H = 32
        Dh = D // H
        qkv = (lambda x, *d: x.transpose(*d))((x @ wqkv).reshape(B, S, 3, H, Dh), 2, 0, 3, 1, 4)
        q, k, v = qkv[0], qkv[1], qkv[2]
        scores = jnp.einsum("bhqd,bhkd->bhqk", q, k) * (Dh ** -0.5)
        p = _softmax(scores, axis=-1)
        o = jnp.einsum("bhqk,bhkd->bhqd", p, v)
        return (lambda x, *d: x.transpose(*d))(o, 0, 2, 1, 3).reshape(B, S, D) @ wo

    def _B_ref(x, w_r, w_gate, w_up, w_down):
        B, S, D = x.shape
        C = 2
        r = x @ w_r
        idx = jnp.argsort(-r, axis=-1)[:, :C]
        idx_e = jnp.repeat(idx.reshape(B, C, 1), D, axis=2)
        x_sel = jnp.take_along_axis(x, idx_e, axis=1)
        g = _silu(x_sel @ w_gate)
        u = x_sel @ w_up
        y = (g * u) @ w_down
        r_sel = _sigmoid(jnp.take_along_axis(r, idx, axis=1))
        y = y * r_sel.reshape(B, C, 1)
        b_off = (jnp.arange(B) * S).reshape(B, 1)
        flat_idx = (idx + b_off).reshape(B * C)
        zero = (x * 0.0).reshape(B * S, D)
        upd = _scatter_add(zero, flat_idx, y.reshape(B * C, D), axis=0)
        return x + upd.reshape(B, S, D)

    x = A_x
    h = x + _A_ref(_layernorm(x, axis=-1), A_wqkv, A_wo)
    h2 = h + _B_ref(_layernorm(h, axis=-1), B_w_r, B_w_gate, B_w_up, B_w_down)
    return h2
```

```python
import math

import jax
import jax.numpy as jnp
from jax import lax
import jax.experimental.pallas as pl
import jax.experimental.pallas.tpu as pltpu

_BF = jnp.bfloat16
_F32 = jnp.float32
_U32 = jnp.uint32

_H = 32
_NQ = 512
_CK = 128
_LAG = 2
_EPS = 1e-5
_NT = (((1,), (1,)), ((), ()))
_TN = (((0,), (0,)), ((), ()))


def _layernorm(v):
    m = jnp.mean(v, axis=-1, keepdims=True)
    c = v - m
    var = jnp.mean(c * c, axis=-1, keepdims=True)
    return c * lax.rsqrt(var + _EPS)


def _rev16(e):
    n = e.shape[0] // 16
    return jnp.concatenate([e[j * 16:(j + 1) * 16] for j in reversed(range(n))], axis=0)


def _pack(v):
    return pltpu.bitcast(v, _U32)


def _unpack(v):
    return pltpu.bitcast(v, _BF)


def _kernel(x_hbm, wqkv_hbm, wo_hbm, wr_ref, wg_hbm, wu_hbm, wd_hbm, out_hbm,
            x_v, wqkv_v, wo_v, wg_v, wu_v, wd_v, wqT, wvT, k_s, qT_s, vT_s, oT_s,
            h_s, out_v, r_s, in_sem, out_sem):
    S, D = x_v.shape
    DH = D // _H
    NB = S // _NQ
    NG = D // 128
    HG = 128 // DH
    NC = S // _CK
    qscale = (DH ** -0.5) * math.log2(math.e)

    x_cp = [pltpu.make_async_copy(x_hbm.at[0, pl.ds(t * _NQ, _NQ)], x_v.at[pl.ds(t * _NQ, _NQ)],
                                  in_sem.at[t]) for t in range(NB)]
    w_cp = [pltpu.make_async_copy(wqkv_hbm.at[:, pl.ds(j * D, D)], wqkv_v.at[:, pl.ds(j * D, D)],
                                  in_sem.at[NB + j]) for j in range(3)]
    o_cp = pltpu.make_async_copy(wo_hbm, wo_v, in_sem.at[NB + 3])
    f_cp = [pltpu.make_async_copy(s, d, in_sem.at[NB + 4 + j])
            for j, (s, d) in enumerate(((wg_hbm, wg_v), (wu_hbm, wu_v), (wd_hbm, wd_v)))]
    x_cp[0].start()
    w_cp[1].start()
    w_cp[2].start()
    w_cp[0].start()
    for c in x_cp[1:]:
        c.start()
    o_cp.start()
    for c in f_cp:
        c.start()

    for t in range(NB):
        x_cp[t].wait()
        ln = _layernorm(x_v[t * _NQ:(t + 1) * _NQ, :].astype(_F32)).astype(_BF)
        if t == 0:
            w_cp[1].wait()
        k = jnp.dot(ln, wqkv_v[:, D:2 * D], preferred_element_type=_F32).astype(_BF)
        k = _pack(k)
        for g in range(NG):
            k_s[g, t * _NQ // 2:(t + 1) * _NQ // 2, :] = k[:, g * 128:(g + 1) * 128]
        if t == 0:
            w_cp[2].wait()
            wvT[...] = _pack(wqkv_v[:, 2 * D:3 * D].T)
        lnr = jnp.concatenate(
            [_rev16(ln[c * _CK:(c + 1) * _CK]) for c in range(_NQ // _CK)], axis=0)
        vT = lax.dot_general(_unpack(wvT[...]), lnr, _NT, preferred_element_type=_F32)
        vT_s[:, t * _NQ:(t + 1) * _NQ] = _pack(vT.astype(_BF))
        if t == 0:
            w_cp[0].wait()
            wqT[...] = _pack(wqkv_v[:, 0:D].T)
        qT = lax.dot_general(_unpack(wqT[...]), ln, _NT, preferred_element_type=_F32)
        qT_s[t] = _pack((qT * qscale).astype(_BF))
    o_cp.wait()

    zero_q = jnp.zeros((DH // 2, _NQ), _U32)

    def q_weights(b, g, j):
        r0 = pl.multiple_of(g * 64 + j * (DH // 2), DH // 2)
        q = qT_s[b, pl.ds(r0, DH // 2), :]
        return _unpack(jnp.concatenate([zero_q] * j + [q] + [zero_q] * (HG - 1 - j), axis=0))

    def group_fast(b, g, carry):
        lmin, lmax = carry
        steps = [(j, c) for j in range(HG) for c in range(NC)]
        st = {}
        pend = {}
        for t in range(len(steps) + _LAG):
            if t < len(steps):
                j, c = steps[t]
                if c == 0:
                    st[j] = [jnp.zeros((8, _NQ), _F32), jnp.zeros((DH, _NQ), _F32)]
                kc = _unpack(k_s[g, c * _CK // 2:(c + 1) * _CK // 2, :])
                s = jnp.dot(kc, q_weights(b, g, j), preferred_element_type=_F32)
                e = jnp.exp2(s)
                st[j][0] = st[j][0] + e.reshape(_CK // 8, 8, _NQ).sum(axis=0)
                pend[t] = _rev16(e).astype(_BF)
            if t >= _LAG:
                j, c = steps[t - _LAG]
                r0 = pl.multiple_of(g * 64 + j * (DH // 2), DH // 2)
                vt = _unpack(vT_s[pl.ds(r0, DH // 2), c * _CK:(c + 1) * _CK])
                st[j][1] = st[j][1] + jnp.dot(vt, pend.pop(t - _LAG), preferred_element_type=_F32)
                if c == NC - 1:
                    l = jnp.sum(st[j][0], axis=0, keepdims=True)
                    o = st[j][1] * (1.0 / l)
                    oT_s[pl.ds(r0, DH // 2), :] = _pack(o.astype(_BF))
                    ok = jnp.logical_and(l > 2.0 ** -30, l < 2.0 ** 60)
                    lmin = jnp.minimum(lmin, jnp.where(ok, 1.0, 0.0))
        return lmin, lmax

    def head_safe(b, hd, _):
        g = hd // HG
        j = hd % HG
        r0 = pl.multiple_of(hd * (DH // 2), DH // 2)
        rg = pl.multiple_of(g * 64, 64)
        qg = _unpack(qT_s[b, pl.ds(rg, 64), :])
        row = lax.broadcasted_iota(jnp.int32, (128, _NQ), 0)
        qw = jnp.where(row // DH == j, qg.astype(_F32), 0.0).astype(_BF)

        def scores(c):
            c0 = pl.multiple_of(c * (_CK // 2), _CK // 2)
            return jnp.dot(_unpack(k_s[g, pl.ds(c0, _CK // 2), :]), qw, preferred_element_type=_F32)

        def pass1(c, m):
            return jnp.maximum(m, jnp.max(scores(c), axis=0, keepdims=True))

        m = lax.fori_loop(0, NC, pass1, jnp.full((1, _NQ), -jnp.inf, _F32))

        def pass2(c, carry):
            l, acc = carry
            e = jnp.exp2(scores(c) - m)
            c0 = pl.multiple_of(c * _CK, _CK)
            vt = _unpack(vT_s[pl.ds(r0, DH // 2), pl.ds(c0, _CK)])
            acc = acc + jnp.dot(vt, _rev16(e).astype(_BF), preferred_element_type=_F32)
            return l + jnp.sum(e, axis=0, keepdims=True), acc

        l, acc = lax.fori_loop(0, NC, pass2,
                               (jnp.zeros((1, _NQ), _F32), jnp.zeros((DH, _NQ), _F32)))
        oT_s[pl.ds(r0, DH // 2), :] = _pack((acc / l).astype(_BF))
        return 0

    def out_copy(b):
        r0 = pl.multiple_of(b * _NQ, _NQ)
        return pltpu.make_async_copy(out_v.at[pl.ds(r0, _NQ)], out_hbm.at[0, pl.ds(r0, _NQ)],
                                     out_sem.at[b])

    def block(b, _):
        one = jnp.ones((1, _NQ), _F32)
        lmin, _unused = lax.fori_loop(0, NG, lambda g, c: group_fast(b, g, c), (one, one))

        @pl.when(jnp.min(lmin) < 0.5)
        def _():
            lax.fori_loop(0, _H, lambda hd, c: head_safe(b, hd, c), 0)

        r0 = pl.multiple_of(b * _NQ, _NQ)
        a = lax.dot_general(_unpack(oT_s[...]), wo_v[...], _TN, preferred_element_type=_F32)
        h = x_v[pl.ds(r0, _NQ), :].astype(_F32) + a
        h_s[pl.ds(r0, _NQ), :] = h
        ln2 = _layernorm(h)
        out_v[pl.ds(r0, _NQ), :] = (h + ln2).astype(_BF)
        out_copy(b).start()
        r = jnp.sum(ln2.astype(_BF).astype(_F32) * wr_ref[...].astype(_F32), axis=-1, keepdims=True)
        lane = lax.broadcasted_iota(jnp.int32, (8, 128), 1)
        rr = jnp.full((8, 128), -jnp.inf, _F32)
        for i in range(_NQ // 8):
            rr = jnp.where(lane == i, r[i * 8:(i + 1) * 8], rr)
        r_s[b] = rr
        return 0

    lax.fori_loop(0, NB, block, 0)

    rr = r_s[...].reshape(NB * 8, 128)
    sub = lax.broadcasted_iota(jnp.int32, rr.shape, 0)
    lane = lax.broadcasted_iota(jnp.int32, rr.shape, 1)
    tok = (sub // 8) * _NQ + lane * 8 + sub % 8
    tok = jnp.where(lane < _NQ // 8, tok, S).astype(_F32)
    rr = jnp.where(rr == rr, rr, -jnp.inf)

    def argtop(vals, cand):
        m = jnp.max(vals, axis=(0, 1), keepdims=True)
        i = jnp.min(jnp.where(vals == m, cand, float(S)), axis=(0, 1), keepdims=True)
        return m, i

    m1, i1 = argtop(rr, tok)
    m2, i2 = argtop(jnp.where(tok == i1, -jnp.inf, rr), jnp.where(tok == i1, float(S), tok))
    t1 = jnp.clip(i1.astype(jnp.int32)[0, 0], 0, S - 1)
    t2 = jnp.clip(i2.astype(jnp.int32)[0, 0], 0, S - 1)
    b1 = pl.multiple_of((t1 // 16) * 16, 16)
    b2 = pl.multiple_of((t2 // 16) * 16, 16)
    hh = jnp.concatenate([h_s[pl.ds(b1, 16), :], h_s[pl.ds(b2, 16), :]], axis=0)
    ln = _layernorm(hh)
    xs = ln.astype(_BF)
    for c in f_cp:
        c.wait()
    gate = jnp.dot(xs, wg_v[...], preferred_element_type=_F32)
    up = jnp.dot(xs, wu_v[...], preferred_element_type=_F32)
    act = (gate * jax.nn.sigmoid(gate) * up).astype(_BF)
    y = jnp.dot(act, wd_v[...], preferred_element_type=_F32)
    base = hh + ln
    for b in range(NB):
        out_copy(b).wait()
    row = lax.broadcasted_iota(jnp.int32, (16, D), 0)
    new1 = (base[:16] + y[:16] * jax.nn.sigmoid(m1)).astype(_BF).astype(_F32)
    out_v[pl.ds(b1, 16), :] = jnp.where(
        row == t1 - b1, new1, out_v[pl.ds(b1, 16), :].astype(_F32)).astype(_BF)
    new2 = (base[16:] + y[16:] * jax.nn.sigmoid(m2)).astype(_BF).astype(_F32)
    out_v[pl.ds(b2, 16), :] = jnp.where(
        row == t2 - b2, new2, out_v[pl.ds(b2, 16), :].astype(_F32)).astype(_BF)
    p1 = pltpu.make_async_copy(out_v.at[pl.ds(b1, 16)], out_hbm.at[0, pl.ds(b1, 16)], out_sem.at[0])
    p2 = pltpu.make_async_copy(out_v.at[pl.ds(b2, 16)], out_hbm.at[0, pl.ds(b2, 16)], out_sem.at[1])
    p1.start()

    @pl.when(b1 != b2)
    def _():
        p2.start()
        p2.wait()

    p1.wait()


@jax.jit
def pallas_sequential_preLN__mha_block__moe_arch_mod__prompt_kernel(
    A_x: jax.Array,
    A_wqkv: jax.Array,
    A_wo: jax.Array,
    B_x: jax.Array,
    B_w_r: jax.Array,
    B_w_gate: jax.Array,
    B_w_up: jax.Array,
    B_w_down: jax.Array,
):
    del B_x
    _, S, D = A_x.shape
    F = B_w_gate.shape[1]
    NB = S // _NQ
    any_spec = pl.BlockSpec(memory_space=pl.ANY)
    return pl.pallas_call(
        _kernel,
        out_shape=jax.ShapeDtypeStruct(A_x.shape, A_x.dtype),
        in_specs=[any_spec, any_spec, any_spec, pl.BlockSpec(memory_space=pltpu.VMEM),
                  any_spec, any_spec, any_spec],
        out_specs=any_spec,
        scratch_shapes=[
            pltpu.VMEM((S, D), _BF),
            pltpu.VMEM((D, 3 * D), _BF),
            pltpu.VMEM((D, D), _BF),
            pltpu.VMEM((D, F), _BF),
            pltpu.VMEM((D, F), _BF),
            pltpu.VMEM((F, D), _BF),
            pltpu.VMEM((D // 2, D), _U32),
            pltpu.VMEM((D // 2, D), _U32),
            pltpu.VMEM((D // 128, S // 2, 128), _U32),
            pltpu.VMEM((NB, D // 2, _NQ), _U32),
            pltpu.VMEM((D // 2, S), _U32),
            pltpu.VMEM((D // 2, _NQ), _U32),
            pltpu.VMEM((S, D), _F32),
            pltpu.VMEM((S, D), _BF),
            pltpu.VMEM((NB, 8, 128), _F32),
            pltpu.SemaphoreType.DMA((NB + 7,)),
            pltpu.SemaphoreType.DMA((NB,)),
        ],
        compiler_params=pltpu.CompilerParams(vmem_limit_bytes=100 * 2 ** 20),
        name="fused_block",
    )(A_x, A_wqkv, A_wo, B_w_r.reshape(1, D), B_w_gate, B_w_up, B_w_down)
```

```python
import math

import jax
import jax.numpy as jnp
from jax import lax
import jax.experimental.pallas as pl
import jax.experimental.pallas.tpu as pltpu

_BF = jnp.bfloat16
_F32 = jnp.float32
_U32 = jnp.uint32

_S, _D, _H = 2048, 512, 32
_DH = _D // _H
_NQ = 512
_NB = _S // _NQ
_NG = _S // 16
_EPS = 1e-5
_NT = (((1,), (1,)), ((), ()))
_TN = (((0,), (0,)), ((), ()))

_P = dict(NV=17, HB=2, SPLIT=1, STUB=0, M3=128, RP=0, PLAG=8, DL=1, VLAG=7, PRE=2, NF=3, NL=1, ROT=0, TAIL=9, HEAD=3, CP=3)
_NV, _HB, _PLAG, _DL, _VLAG, _PRE, _NF, _NL = (
    _P[k] for k in ("NV", "HB", "PLAG", "DL", "VLAG", "PRE", "NF", "NL"))
_NA = 2


def _plan():
    period = _NG + _NG // 8 - _NV
    pv = [math.ceil((t + 1) * period / 16 + _PLAG + _DL) for t in range(16)]
    busy = {p % period for p in pv}
    assert len(busy) == 16
    qk = [s for s in range(period) if s not in busy]
    dslot = [math.floor(_VLAG + i * period / (_DH * _NV)) for i in range(_DH * _NV)]
    ev = [(s + _PLAG + 0.5, ("m", m)) for m, s in enumerate(qk)]
    ev += [(dslot[_DH * v + _DH - 1], ("v", v)) for v in range(_NV)]
    ev.sort(key=lambda e: e[0])
    assert all(ev[8 * t + 7][0] < pv[t] for t in range(16))
    blk = {ev[i][1]: 8 * (i // 8) + 7 - i % 8 for i in range(_NG)}
    return period, pv, qk, dslot, blk


_PERIOD, _PV, _QK, _DSLOT, _BLK = _plan()

_A_KB = 0
_A_QB = _A_KB + 8 * _NV
_A_K = _A_QB + _NB * _DH
_A_V = _A_K + _NG // 4
_A_Q = _A_V + _NB
_A_C = _A_Q + _NB
_A_O = _A_C + 10
_A_F = _A_O + 2
_A_ROWS = _A_F + 3
_NVC = -(-_NV // 8)
_R_K = 0
_R_Q = _R_K + _NG
_R_V = _R_Q + 2 * _H * _NB
_R_KV = _R_V + _H * _NB
_R_F = _R_KV + 2 * _H
_R_ROWS = _R_F + 1


def _layernorm(v):
    m = jnp.mean(v, axis=-1, keepdims=True)
    c = v - m
    var = jnp.mean(c * c, axis=-1, keepdims=True)
    return c * lax.rsqrt(var + _EPS)


def _pack(v):
    return pltpu.bitcast(v, _F32)


def _unpack(v):
    return pltpu.bitcast(v, _BF)


def _lt(n):
    return slice(n * 128, (n + 1) * 128)


def _prep_jobs(src, dst, hd, z):
    grp = 0 if isinstance(hd, int) else pl.multiple_of((hd // 8) * 128, 128)
    shift = (128 - _DH * (hd % 8)) % 128

    def k_job(m):
        w = pltpu.bitcast(src[z + (_R_K + _BLK["m", m]), :, pl.ds(grp, 128)], _U32)
        dst[(_QK[m] - _PRE) % _PERIOD % _NA][_A_K + m // 4, :, _lt(m % 4)] = pltpu.bitcast(
            w if isinstance(hd, int) else pltpu.roll(w, shift, 1), _F32)

    def kb_job(d, c):
        n = min(8, _NV - 8 * c)
        k = src[z + (_R_KV + 2 * hd + d // 8), :, _lt(c)][d % 8:d % 8 + 1, :16 * n]
        kb = jnp.broadcast_to(k, (128, 16 * n)).T
        for i in range(n):
            v = 8 * c + i
            a = dst[_DSLOT[_DH * v + d] % _PERIOD % _NA]
            for r in range(2):
                a[_A_KB + 8 * v + d // 2, :, _lt(2 * (d % 2) + r)] = kb[
                    16 * i + 8 * r:16 * i + 8 * r + 8]

    def qb_job(b, d, n):
        q = src[z + (_R_Q + (2 * hd + d // 8) * _NB + b), :, 256 * n:256 * (n + 1)]
        qb = jnp.broadcast_to(q[d % 8:d % 8 + 1], (8, 256))
        for i in {_DSLOT[_DH * v + d] % _PERIOD % _NA for v in range(_NV)}:
            dst[i][_A_QB + b * _DH + d, :, 256 * n:256 * (n + 1)] = qb

    def qv_job(b):
        q = jnp.concatenate([src[z + (_R_Q + (2 * hd + i) * _NB + b)] for i in range(2)], axis=0)
        q = _pack(q.astype(_BF))
        v = src[z + (_R_V + hd * _NB + b)]
        for a in dst:
            a[_A_Q + b] = q
            a[_A_V + b] = v

    jobs = [(i / (_NG - _NV), k_job, (i,)) for i in range(_NG - _NV)]
    jobs += [(i / (_NVC * _DH), kb_job, divmod(i, _NVC)) for i in range(_NVC * _DH)]
    jobs += [((i + 0.5) / (2 * _DH * _NB), qb_job, (i // (2 * _DH), i // 2 % _DH, i % 2))
             for i in range(2 * _DH * _NB)]
    jobs += [((i + 0.5) / _NB, qv_job, (i,)) for i in range(_NB)]
    return sorted(jobs, key=lambda j: j[0])


def _finish(o, den, hd, b, oT_s, den_s):
    l = jnp.sum(den, axis=0, keepdims=True)
    inv = pltpu.reciprocal(l, approx=True)
    inv = inv * (2.0 - l * inv)
    oT_s[b, pl.ds(pl.multiple_of(hd * 8, 8), 8), :] = _pack((o * inv).astype(_BF))
    den_s[pl.ds(hd * _NB + b, 1), :] = l


def _attend(hd0, nh, parity, src, arenas, oT_s, den_s):
    zl, zs = hd0 // _H, hd0 // (2 * _H)
    units = nh * _NB
    mx, vp, prep = {}, {}, {}
    for u in range(units):
        for m, s in enumerate(_QK):
            mx[u * _PERIOD + s] = ("qk", u, m)
        for t, s in enumerate(_PV):
            mx[u * _PERIOD + s] = ("pv", u, t)
        for i, s in enumerate(_DSLOT):
            vp.setdefault(u * _PERIOD + s, []).append((u, i // _DH, i % _DH))
    del mx[(units - 1) * _PERIOD + _PV[15]]
    mx[_PV[15] - _PERIOD] = ("pv", -1, 15)
    for j in range(nh):
        first, span = j * _NB * _PERIOD + _P["HEAD"] * 8, _NB * _PERIOD - _P["TAIL"] * 8
        for frac, job, args in _prep_jobs(src, arenas[(parity + j + 1) % 2],
                                          jnp.minimum(hd0 + j + 1, _H - 1), zl):
            prep.setdefault(first + int(frac * span), []).append((job, args))
    runs, run = {}, []
    for s in sorted(mx):
        if run and mx[s][:2] != mx[run[0]][:2]:
            runs[run[-1]] = run
            run = []
        if mx[s][0] == "qk":
            run.append(s)
    starts = {}
    for r in runs.values():
        starts.setdefault(runs[r[0] - 1][0] if r[0] - 1 in runs else r[0], []).append(r[0])

    def arena(u, s):
        return arenas[(parity + max(u, 0) // _NB) % 2][s % _PERIOD % _NA]

    carry = arenas[(parity + nh) % 2][0]
    den, acc, lhs, rhs, res, prob = {}, {-1: arenas[parity][0]}, {}, {}, {}, {}

    def emit(u, scores, key):
        e = jnp.exp2(scores)
        t = e[:8] + e[8:]
        den[u] = den[u] + t if u in den else t
        if u == units - 1 and _BLK[key] >= _NG - 8:
            carry[_A_C + _BLK[key] % 8] = _pack(e.astype(_BF))
        else:
            prob[u, _BLK[key]] = e

    vacc = last = vlast = None
    for s in range(-_PRE, units * _PERIOD + 2 * _PLAG + _DL):
        if mx.get(s + _P["CP"], (0, 0))[1] == -1:
            rhs[-1] = _unpack(jnp.concatenate([acc[-1][zl + (_A_C + g)] for g in range(8)], axis=0))
        if s + _PRE in mx:
            kind, u, i = mx[s + _PRE]
            a = arena(u, s)
            if kind == "qk":
                for r in starts.get(s + _PRE, []):
                    rhs[r] = _unpack(arena(mx[r][1], s)[zl + (_A_Q + mx[r][1] % _NB)])
                lhs[s + _PRE] = a[zl + (_A_K + i // 4), :, _lt(i % 4)]
            elif u < 0:
                lhs[s + _PRE] = acc[u][zl + (_A_C + 8), :, _lt(0)]
            else:
                lhs[s + _PRE] = a[zl + (_A_V + i // 4), :, _lt(i % 4)]
        for u, v, d in vp.get(s, []):
            a = arena(u, s)
            kb = [a[zl + (_A_KB + 8 * v + d // 2), :, _lt(2 * (d % 2) + r)] for r in range(2)]
            kb = jnp.concatenate([jnp.concatenate([k] * 4, axis=1) for k in kb], axis=0)
            qb = a[zl + (_A_QB + (u % _NB) * _DH + d)]
            pr = kb * jnp.concatenate([qb, qb], axis=0)
            vacc = pr if d == 0 else vacc + pr
            vlast = u
            if d == _DH - 1:
                emit(u, vacc, ("v", v))
        for job, args in prep.get(s, []):
            job(*args)
        if s in runs:
            k = _unpack(jnp.concatenate([lhs[r] for r in runs[s]], axis=0))[:, :_DH]
            sc = jnp.dot(k, rhs[runs[s][0]], preferred_element_type=_F32)
            for i, r in enumerate(runs[s]):
                res[r] = sc[16 * i:16 * (i + 1)]
        elif s in mx and mx[s][0] == "pv":
            _, u, t = mx[s]
            p = rhs[u] if u < 0 else jnp.concatenate(
                [prob.pop((u, 8 * t + g)) for g in range(8)], axis=0)
            res[s] = jnp.dot(_unpack(lhs[s]), p, preferred_element_type=_F32)
        for r in [r for r in sorted(res) if r + _PLAG <= s]:
            kind, u, i = mx[r]
            val = res.pop(r)
            if kind == "qk":
                last = u
                emit(u, val, ("m", i))
                continue
            if i > 0:
                val = jnp.concatenate([acc[u][zl + (_A_O + n)] for n in range(2)], axis=0) + val
            if u < 0:
                prev = jnp.where(hd0 > 0, hd0 - 1, _H)
                _finish(val, acc[u][zl + (_A_C + 9)], prev, _NB - 1, oT_s, den_s)
            elif i == 15:
                _finish(val, den[u], hd0 + u // _NB, u % _NB, oT_s, den_s)
            elif u == units - 1 and i == 14:
                carry[_A_O] = val[:8]
                carry[_A_O + 1] = val[8:]
            else:
                acc[u] = arena(u, s)
                acc[u][zs + _A_O] = val[:8]
                acc[u][zs + (_A_O + 1)] = val[8:]
        if last is not None and s < units * _PERIOD:
            for i in range(_NL):
                n = (s * _NL + i) % 4
                arena(last, s)[zs + _A_F, :, _lt(n)] = den[last][:, _lt(n)]
            if s in prep:
                src[zs + _R_F, :, _lt(0)] = den[last][:, _lt(0)]
        if s in vp:
            for i in range(_NF):
                n = (s * _NF + i + s // 2 * _P["ROT"] * _NF) % 8
                arena(vlast, s)[zs + (_A_F + 1 + n // 4), :, _lt(n % 4)] = vacc[
                    8 * (n // 4):8 * (n // 4) + 8, _lt(n % 4)]
    assert not res and not prob
    carry[_A_C + 8, :, _lt(0)] = arena(units - 1, 0)[zl + (_A_V + _NB - 1), :, _lt(3)]
    carry[_A_C + 9] = den[units - 1]


def _attend_all(src, arenas, oT_s, den_s):
    first = arenas[0][0]
    first[pl.ds(_A_C, _A_F - _A_C)] = jnp.ones((_A_F - _A_C, 8, _NQ), _F32)

    @pl.loop(0, _H // _HB)
    def _(it):
        if _P["SPLIT"]:
            for j in range(_HB):
                pl.when(it < _H - j)(
                    lambda: _attend(it * _HB + j, 1, j % 2, src, arenas, oT_s, den_s))
        else:
            _attend(it * _HB, _HB, 0, src, arenas, oT_s, den_s)

    p = _unpack(jnp.concatenate([first[_A_C + g] for g in range(8)], axis=0))
    o = jnp.dot(_unpack(first[_A_C + 8, :, _lt(0)]), p, preferred_element_type=_F32)
    o = o + jnp.concatenate([first[_A_O], first[_A_O + 1]], axis=0)
    _finish(o, first[_A_C + 9], _H - 1, _NB - 1, oT_s, den_s)


def _attend_safe(i, src, oT_s):
    hd, b = i // _NB, i % _NB
    grp = pl.multiple_of((hd // 8) * 128, 128)
    q = jnp.concatenate([src[_R_Q + (2 * hd + n) * _NB + b] for n in range(2)], axis=0)
    row = lax.broadcasted_iota(jnp.int32, (128, _NQ), 0)
    qw = jnp.where(row // _DH == hd % 8, jnp.concatenate([q] * 8, axis=0), 0.0).astype(_BF)

    def scores(c):
        k = src[pl.ds(_R_K + 32 * c, 32), :, pl.ds(grp, 128)].reshape(256, 128)
        return jnp.dot(_unpack(k), qw, preferred_element_type=_F32)

    def pass1(c, m):
        return jnp.maximum(m, jnp.max(scores(c), axis=0, keepdims=True))

    m = lax.fori_loop(0, _NB, pass1, jnp.full((1, _NQ), -jnp.inf, _F32))

    def pass2(c, carry):
        e = jnp.exp2(scores(c) - m)
        v = _unpack(src[_R_V + hd * _NB + c])
        return (carry[0] + jnp.sum(e, axis=0, keepdims=True),
                carry[1] + jnp.dot(v, e.astype(_BF), preferred_element_type=_F32))

    l, o = lax.fori_loop(0, _NB, pass2,
                         (jnp.zeros((1, _NQ), _F32), jnp.zeros((_DH, _NQ), _F32)))
    oT_s[b, pl.ds(pl.multiple_of(hd * 8, 8), 8), :] = _pack((o / l).astype(_BF))


def _kernel(x_hbm, wqkv_hbm, wo_hbm, wr_ref, wg_hbm, wu_hbm, wd_hbm, out_hbm,
            x_v, wqkv_v, wo_v, wg_v, wu_v, wd_v, wqT, wvT, wo_p, src, oT_s,
            den_s, ln_s, base_s, out_v, fix_v, in_sem, out_sem, *stage):
    S, D = _S, _D
    arenas = (stage[:_NA], stage[_NA:])
    qscale = (_DH ** -0.5) * math.log2(math.e)

    def rows(t):
        return pl.ds(t * _NQ, _NQ)

    x_cp = [pltpu.make_async_copy(x_hbm.at[0, rows(t)], x_v.at[rows(t)], in_sem.at[t])
            for t in range(_NB)]
    w_cp = [pltpu.make_async_copy(wqkv_hbm.at[:, pl.ds(j * D, D)], wqkv_v.at[:, pl.ds(j * D, D)],
                                  in_sem.at[_NB + j]) for j in range(3)]
    o_cp = pltpu.make_async_copy(wo_hbm, wo_v, in_sem.at[_NB + 3])
    f_cp = [pltpu.make_async_copy(s, d, in_sem.at[_NB + 4 + j])
            for j, (s, d) in enumerate(((wg_hbm, wg_v), (wu_hbm, wu_v), (wd_hbm, wd_v)))]
    for c in [x_cp[0], w_cp[1], x_cp[1], w_cp[2], w_cp[0], x_cp[2], x_cp[3]]:
        c.start()

    ln, kv = {}, [jnp.zeros((16, D), _F32)] * (8 * _NVC)
    vmax = [jnp.zeros((8, _NQ), _F32)]

    def ln1(t):
        ln[t] = _layernorm(x_v[rows(t), :].astype(_F32)).astype(_BF)

    def proj_k(t, lo=0, n=32):
        k = jnp.dot(ln[t][16 * lo:16 * (lo + n)], wqkv_v[:, D:2 * D], preferred_element_type=_F32)
        src[pl.ds(_R_K + 32 * t + lo, n)] = _pack(k.astype(_BF)).reshape(n, 8, D)
        for v in range(_NV):
            g = _BLK["v", v] - 32 * t - lo
            if 0 <= g < n:
                kv[v] = k[16 * g:16 * g + 16]

    def proj_v(t):
        vT = lax.dot_general(_unpack(wvT[...]), ln[t], _NT, preferred_element_type=_F32)
        vmax[0] = jnp.maximum(vmax[0], jnp.max(jnp.abs(vT).reshape(D // 8, 8, _NQ), axis=0))
        vT = _pack(vT.astype(_BF))
        for hd in range(_H):
            src[_R_V + hd * _NB + t] = vT[8 * hd:8 * hd + 8]

    def proj_q(t, lo, n):
        qT = lax.dot_general(_unpack(wqT[4 * lo:4 * (lo + n)]), ln[t], _NT,
                             preferred_element_type=_F32) * qscale
        for i in range(n):
            src[_R_Q + (lo + i) * _NB + t] = qT[8 * i:8 * i + 8]

    x_cp[0].wait()
    w_cp[1].wait()
    ln1(0)
    proj_k(0, 0, 16)
    x_cp[1].wait()
    w_cp[2].wait()
    proj_k(0, 16, 16)
    ln1(1)
    wvT[...] = _pack(wqkv_v[:, 2 * D:3 * D].T)
    proj_k(1)
    for c in (w_cp[0], x_cp[2], x_cp[3]):
        c.wait()
    for c in [o_cp] + f_cp:
        c.start()
    proj_v(0)
    ln1(2)
    wqT[...] = _pack(wqkv_v[:, 0:D].T)
    proj_v(1)
    ln1(3)
    proj_k(2)
    proj_k(3)
    src[pl.ds(_R_KV, 2 * _H), :, :128 * _NVC] = jnp.concatenate(kv, axis=0).T.reshape(
        2 * _H, 8, 128 * _NVC)
    proj_v(2)
    proj_v(3)
    for t in range(_NB):
        proj_q(t, 0, 2 * _H)
    vmax = vmax[0]

    for _, job, args in _prep_jobs(src, arenas[0], 0, 0):
        job(*args)
    if not _P["STUB"]:
        _attend_all(src, arenas, oT_s, den_s)
    else:
        for a in arenas[0]:
            den_s[:8] = a[vmax[0, 0].astype(jnp.int32)]
    den = den_s[:_H * _NB]
    ok = jnp.where(den > 2.0 ** -30, jnp.where(den < 2.0 ** 60, 1.0, 0.0), 0.0)
    ok = jnp.where(vmax < 2.0 ** 60, jnp.min(ok.reshape(-1, 8, _NQ), axis=0), 0.0)

    for c in [o_cp] + f_cp:
        c.wait()
    if _P["RP"]:
        wo_p[...] = _pack(wo_v[...])

    @pl.when(jnp.min(ok) < 0.5)
    def _():
        pl.loop(0, _H * _NB)(lambda i: _attend_safe(i, src, oT_s))

    half = [pl.ds(i * S // 2, S // 2) for i in range(2)]
    out_cp = [pltpu.make_async_copy(out_v.at[half[i]], out_hbm.at[0, half[i]], out_sem.at[i])
              for i in range(2)]
    wr = wr_ref[...].astype(_F32).reshape(1, D)
    lane = lax.broadcasted_iota(jnp.int32, (8, 128), 1)
    rr = [jnp.zeros((8, 128), _F32)] * 2
    n = _P["M3"]
    for lo in range(0, S, n):
        if lo % 128 == 0:
            o = _pack(_unpack(oT_s[lo // _NQ, :D // 2, lo % _NQ:lo % _NQ + max(n, 128)]).T)
        a = jnp.dot(_unpack(o[lo % 128 // 2:(lo % 128 + n) // 2]), _unpack(wo_p[...]) if _P["RP"] else wo_v[...],
                    preferred_element_type=_F32)
        if lo == S // 2 + 256:
            out_cp[0].start()
        h = x_v[lo:lo + n, :].astype(_F32) + a
        c = h - jnp.mean(h, axis=-1, keepdims=True)
        rstd = lax.rsqrt(jnp.mean(c * c, axis=-1, keepdims=True) + _EPS)
        r = jnp.sum(c * wr, axis=-1, keepdims=True) * rstd
        ln2 = c * rstd
        base = h + ln2
        ln_s[lo:lo + n, :] = ln2
        base_s[lo:lo + n, :] = base
        out_v[lo:lo + n, :] = base.astype(_BF)
        for i in range(n // 8):
            j, k = divmod(lo // 8 + i, 128)
            rr[j] = jnp.where(lane == k, r[8 * i:8 * i + 8], rr[j])
    out_cp[1].start()

    rr = jnp.concatenate(rr, axis=0)
    sub = lax.broadcasted_iota(jnp.int32, rr.shape, 0)
    lane = lax.broadcasted_iota(jnp.int32, rr.shape, 1)
    tok = ((sub // 8) * 1024 + lane * 8 + sub % 8).astype(_F32)
    rr = jnp.where(rr == rr, rr, -jnp.inf)
    m1 = jnp.max(rr, axis=(0, 1), keepdims=True)
    i1 = jnp.min(jnp.where(rr == m1, tok, S), axis=(0, 1), keepdims=True)
    m2 = jnp.max(jnp.where(rr == m1, -jnp.inf, rr), axis=(0, 1), keepdims=True)
    i2 = jnp.where(rr == m1, jnp.where(tok == i1, 2 * S, tok), jnp.where(rr == m2, tok + S, 2 * S))
    i2 = jnp.min(i2, axis=(0, 1), keepdims=True)
    m2 = jnp.where(i2 < S, m1, m2)
    t1 = i1.astype(jnp.int32)[0, 0] & (S - 1)
    t2 = i2.astype(jnp.int32)[0, 0] & (S - 1)
    b1 = pl.multiple_of(t1 & (S - 16), 16)
    b2 = pl.multiple_of(t2 & (S - 16), 16)
    xs = jnp.concatenate([ln_s[pl.ds(b1, 16), :], ln_s[pl.ds(b2, 16), :]], axis=0).astype(_BF)
    gate = jnp.dot(xs, wg_v[...], preferred_element_type=_F32)
    up = jnp.dot(xs, wu_v[...], preferred_element_type=_F32)
    act = (gate * jax.nn.sigmoid(gate) * up).astype(_BF)
    y = jnp.dot(act, wd_v[...], preferred_element_type=_F32)
    row = lax.broadcasted_iota(jnp.int32, (16, D), 0)
    y1 = y[:16] * jax.nn.sigmoid(m1)
    y2 = y[16:] * jax.nn.sigmoid(m2)
    for i, b in enumerate((b1, b2)):
        upd = jnp.where(row == t1 - b, y1, jnp.where(row == t2 - b, y2, 0.0))
        fix_v[i] = (base_s[pl.ds(b, 16), :] + upd).astype(_BF)
    for c in out_cp:
        c.wait()
    p1 = pltpu.make_async_copy(fix_v.at[0], out_hbm.at[0, pl.ds(b1, 16)], out_sem.at[0])
    p2 = pltpu.make_async_copy(fix_v.at[1], out_hbm.at[0, pl.ds(b2, 16)], out_sem.at[1])
    p1.start()

    @pl.when(b1 != b2)
    def _():
        p2.start()
        p2.wait()

    p1.wait()


@jax.jit
def pallas_sequential_preLN__mha_block__moe_arch_mod__prompt_kernel(
    A_x: jax.Array,
    A_wqkv: jax.Array,
    A_wo: jax.Array,
    B_x: jax.Array,
    B_w_r: jax.Array,
    B_w_gate: jax.Array,
    B_w_up: jax.Array,
    B_w_down: jax.Array,
):
    del B_x
    S, D = _S, _D
    assert A_x.shape == (1, S, D)
    F = B_w_gate.shape[1]
    any_spec = pl.BlockSpec(memory_space=pl.ANY)
    return pl.pallas_call(
        _kernel,
        out_shape=jax.ShapeDtypeStruct(A_x.shape, A_x.dtype),
        in_specs=[any_spec, any_spec, any_spec, pl.BlockSpec(memory_space=pltpu.VMEM),
                  any_spec, any_spec, any_spec],
        out_specs=any_spec,
        scratch_shapes=[
            pltpu.VMEM((S, D), _BF),
            pltpu.VMEM((D, 3 * D), _BF),
            pltpu.VMEM((D, D), _BF),
            pltpu.VMEM((D, F), _BF),
            pltpu.VMEM((D, F), _BF),
            pltpu.VMEM((F, D), _BF),
            pltpu.VMEM((D // 2, D), _F32),
            pltpu.VMEM((D // 2, D), _F32),
            pltpu.VMEM((D // 2, D), _F32),
            pltpu.VMEM((_R_ROWS, 8, _NQ), _F32),
            pltpu.VMEM((_NB, D // 2 + 8, _NQ), _F32),
            pltpu.VMEM(((_H + 2) * _NB, _NQ), _F32),
            pltpu.VMEM((S, D), _F32),
            pltpu.VMEM((S, D), _F32),
            pltpu.VMEM((S, D), _BF),
            pltpu.VMEM((2, 16, D), _BF),
            pltpu.SemaphoreType.DMA((_NB + 7,)),
            pltpu.SemaphoreType.DMA((2,)),
        ] + [pltpu.VMEM((_A_ROWS, 8, _NQ), _F32)] * (2 * _NA),
        compiler_params=pltpu.CompilerParams(vmem_limit_bytes=100 * 2 ** 20),
        name="fused_block",
    )(A_x, A_wqkv, A_wo, B_w_r, B_w_gate, B_w_up, B_w_down)
```

```python
import math

import jax
import jax.numpy as jnp
from jax import lax
import jax.experimental.pallas as pl
import jax.experimental.pallas.tpu as pltpu

_BF = jnp.bfloat16
_F32 = jnp.float32

_S, _D, _H = 2048, 512, 32
_DH = _D // _H
_EPS = 1e-5
_NQ = 512
_NB = _S // _NQ
_NG = _S // 16
_NV = 20
_NU = 2 * _NB
_NBUF = 8
_NT = (((1,), (1,)), ((), ()))

_RESULT_LAG = 7
_TILE_LAG = 2
_VPU_LAG = 4
_FETCH_LEAD = 3
_PACE_LEAD = 3


def _plan():
    period = _NG + _NG // 8 - _NV
    pv = [math.ceil((t + 1) * period / 16 + _RESULT_LAG + _TILE_LAG) for t in range(16)]
    busy = [s % period for s in pv]
    qk = [s for s in range(period) if s not in busy]
    step = [math.floor(_VPU_LAG + i * period / (_DH * _NV)) for i in range(_DH * _NV)]
    done = [(s + _RESULT_LAG + 0.5, "mxu", m) for m, s in enumerate(qk)]
    done += [(step[_DH * v + _DH - 1], "vpu", v) for v in range(_NV)]
    done.sort()
    assert len(done) == _NG and all(done[8 * t + 7][0] < pv[t] for t in range(16))
    group = {e[1:]: i ^ 7 for i, e in enumerate(done)}
    ops, steps = {pv[15] - period: ("pv", -1, 15)}, {}
    for u in range(_NU):
        ops.update({u * period + s: ("qk", u, group["mxu", m]) for m, s in enumerate(qk)})
        ops.update({u * period + s: ("pv", u, t) for t, s in enumerate(pv)})
        for i, s in enumerate(step):
            steps.setdefault(u * period + s, []).append((u,) + divmod(i, _DH))
    del ops[(_NU - 1) * period + pv[15]]
    return period, ops, steps, [group["vpu", v] for v in range(_NV)]


def _runs(ops):
    runs, run = {}, []
    for s in sorted(ops):
        if run and ops[s][:2] != ops[run[0]][:2]:
            runs[run[-1]] = run
            run = []
        if ops[s][0] == "qk":
            run.append(s)
    starts = {}
    for r in runs.values():
        starts.setdefault(runs[r[0] - 1][0] if r[0] - 1 in runs else r[0], []).append(r[0])
    return runs, starts


_PERIOD, _OPS, _STEPS, _VPU_GROUPS = _plan()
_RUNS, _STARTS = _runs(_OPS)

_KT = -(-_NV // 8)
_R_K = 0
_R_Q = _R_K + _NG
_R_V = _R_Q + 2 * _H * _NB
_R_QP = _R_V + _H * _NB
_R_KT = _R_QP + _H * _NB
_R_PACE = _R_KT + 2 * _H
_R_ROWS = _R_PACE + 1
_ND = _DH // _NBUF
_A_KB = 0
_A_QB = _A_KB + _ND * (_NV + 1) // 2
_A_K = _A_QB + _NB * _ND
_A_V = _A_K + _NG // 4
_A_Q = _A_V + _NB
_A_LAST = _A_Q + _NB
_A_PACE = _A_LAST + 12
_A_ROWS = _A_PACE + 4


def _layernorm(v):
    c = v - jnp.mean(v, axis=-1, keepdims=True)
    return c * lax.rsqrt(jnp.mean(c * c, axis=-1, keepdims=True) + _EPS)


def _pack(v):
    return pltpu.bitcast(v, _F32)


def _unpack(v):
    return pltpu.bitcast(v, _BF)


def _lanes(n):
    return slice(n * 128, (n + 1) * 128)


def _swap_halves(v):
    return jnp.concatenate(
        [v[8 * (i ^ 1):8 * (i ^ 1) + 8] for i in range(v.shape[0] // 8)], axis=0)


def _mxu_buf(s):
    return _STEPS[s % _PERIOD + _PERIOD][-1][2] % _NBUF


def _staging_jobs(proj, dst, hd, z):
    static = isinstance(hd, int)
    assert not static or hd == 0
    lane0 = 0 if static else pl.multiple_of((hd >> 3) * 128, 128)
    shift = (128 - _DH * (hd & 7)) & 127
    k_use, q_use, v_use = {}, {}, {}
    for s, (kind, _, i) in _OPS.items():
        (k_use if kind == "qk" else v_use).setdefault(i, set()).add(_mxu_buf(s - _FETCH_LEAD))
    for s, firsts in _STARTS.items():
        for r in firsts:
            q_use.setdefault(_OPS[r][1] % _NB, set()).add(_mxu_buf(s - _FETCH_LEAD))

    def k_job(g):
        k = proj[z + (_R_K + g), :, pl.ds(lane0, 128)]
        if not static:
            k = pltpu.bitcast(pltpu.roll(pltpu.bitcast(k, jnp.uint32), shift, 1), _F32)
        for i in sorted(k_use[g]):
            dst[i][_A_K + g // 4, :, _lanes(g % 4)] = k

    def kb_job(d, c):
        n = min(8, _NV - 8 * c)
        k = proj[z + (_R_KT + 2 * hd + d // 8), :, _lanes(c)][d % 8:d % 8 + 1, :16 * n]
        kb = jnp.broadcast_to(k, (128, 16 * n)).T
        for r in range(2 * n):
            v = 8 * c + r // 2
            dst[d % _NBUF][_A_KB + v // 2 * _ND + d // _NBUF, :, _lanes(2 * (v % 2) + r % 2)] = (
                kb[8 * r:8 * r + 8])

    def qb_job(b, d, n):
        cols = slice(256 * n, 256 * (n + 1))
        q = proj[z + (_R_Q + (2 * hd + d // 8) * _NB + b), :, cols]
        dst[d % _NBUF][_A_QB + b * _ND + d // _NBUF, :, cols] = jnp.broadcast_to(
            q[d % 8:d % 8 + 1], (8, 256))

    def q_job(b, n):
        q = proj[z + (_R_QP + hd * _NB + b), :, _lanes(n)]
        for i in sorted(q_use[b]):
            dst[i][_A_Q + b, :, _lanes(n)] = q

    def v_job(b, n):
        v = proj[z + (_R_V + hd * _NB + b), :, _lanes(n)]
        for i in sorted(v_use[4 * b + n]):
            dst[i][_A_V + b, :, _lanes(n)] = v

    jobs = [(i / len(k_use), k_job, (g,)) for i, g in enumerate(sorted(k_use))]
    jobs += [(i / (_KT * _DH), kb_job, divmod(i, _KT)) for i in range(_KT * _DH)]
    jobs += [((i + 0.5) / (2 * _DH * _NB), qb_job, (i // (2 * _DH), i // 2 % _DH, i % 2))
             for i in range(2 * _DH * _NB)]
    jobs += [((i + 0.25) / 16, q_job, divmod(i, 4)) for i in range(16)]
    jobs += [((i + 0.75) / 16, v_job, divmod(i, 4)) for i in range(16)]
    return sorted(jobs, key=lambda job: job[0])


def _normalize(o, den, hd, b, o_t, den_s):
    total = jnp.sum(den, axis=0, keepdims=True)
    inv = pltpu.reciprocal(total, approx=True)
    inv = inv * (2.0 - total * inv)
    o_t[b, pl.ds(pl.multiple_of(hd * 8, 8), 8), :] = _pack((o * inv).astype(_BF))
    den_s[pl.ds(hd * _NB + b, 1), :] = total


def _attend_pair(hd, proj, bufs, o_t, den_s):
    zl, zs = hd >> 5, hd >> 6
    staging, end = {}, max(_OPS)
    for j in range(2):
        for t, job, args in _staging_jobs(proj, bufs[1 - j], jnp.minimum(hd + j + 1, _H - 1), zl):
            s = j * _NB * _PERIOD + 16 + int(t * (_NB * _PERIOD - 40))
            staging.setdefault(s, []).append((job, args))
    handoff = bufs[0][0]
    den, acc, lhs, rhs, res, prob = {}, {}, {}, {}, {}, {}

    def buf(u, i):
        return bufs[min(u, _NU - 1) // _NB][i % _NBUF]

    def exponentiate(u, g, scores):
        e = jnp.exp2(scores)
        den[u] = den[u] + (e[:8] + e[8:]) if u in den else e[:8] + e[8:]
        e = _swap_halves(e)
        if u == _NU - 1 and g >= _NG - 8:
            handoff[_A_LAST + g % 8] = _pack(e.astype(_BF))
        else:
            prob[u, g] = e

    part = last = None
    n_steps = n_paced = 0
    for s in range(-_FETCH_LEAD, max(end + _RESULT_LAG, max(_STEPS)) + 1):
        if s + _FETCH_LEAD in _OPS:
            kind, u, i = _OPS[s + _FETCH_LEAD]
            if kind == "qk":
                for r in _STARTS.get(s + _FETCH_LEAD, []):
                    w = _OPS[r][1]
                    rhs[r] = _unpack(buf(w, _mxu_buf(s))[zl + (_A_Q + w % _NB)])
                operand = buf(u, _mxu_buf(s))[zl + (_A_K + i // 4), :, _lanes(i % 4)]
            elif u < 0:
                rhs[u] = _unpack(
                    jnp.concatenate([handoff[zl + (_A_LAST + g)] for g in range(8)], axis=0))
                operand = handoff[zl + (_A_LAST + 8), :, _lanes(0)]
            else:
                operand = buf(u, _mxu_buf(s))[zl + (_A_V + i // 4), :, _lanes(i % 4)]
            lhs[s + _FETCH_LEAD] = operand

        for u, v, d in _STEPS.get(s, []):
            kb = [buf(u, d)[zl + (_A_KB + v // 2 * _ND + d // _NBUF), :, _lanes(2 * (v % 2) + r)]
                  for r in range(2)]
            kb = jnp.concatenate([jnp.concatenate([k] * 4, axis=1) for k in kb], axis=0)
            qb = buf(u, d)[zl + (_A_QB + u % _NB * _ND + d // _NBUF)]
            term = kb * jnp.concatenate([qb, qb], axis=0)
            part = term if d == 0 else part + term
            ahead = d + _PACE_LEAD
            for _ in range(1 if n_steps % 3 else 2):
                r, n = divmod(n_paced % 8, 4)
                buf(u + (v + ahead // _DH) // _NV, ahead)[zs + (_A_PACE + 1 + r), :, _lanes(n)] = (
                    part[8 * r:8 * r + 8, _lanes(n)])
                n_paced += 1
            n_steps += 1
            if d == _DH - 1:
                exponentiate(u, _VPU_GROUPS[v], part)

        for job, args in staging.get(s, []):
            job(*args)

        if s in _RUNS:
            k = _unpack(jnp.concatenate([lhs[r] for r in _RUNS[s]], axis=0))[:, :_DH]
            scores = jnp.dot(k, rhs[_RUNS[s][0]], preferred_element_type=_F32)
            for i, r in enumerate(_RUNS[s]):
                res[r] = scores[16 * i:16 * (i + 1)]
        elif s in _OPS and _OPS[s][0] == "pv":
            _, u, t = _OPS[s]
            p = rhs[u] if u < 0 else jnp.concatenate(
                [prob.pop((u, 8 * t + g)) for g in range(8)], axis=0)
            res[s] = jnp.dot(_unpack(lhs[s]), p, preferred_element_type=_F32)

        paced = buf((s + _PACE_LEAD) // _PERIOD, _mxu_buf(s + _PACE_LEAD))
        for r in [r for r in sorted(res) if r + _RESULT_LAG <= s]:
            kind, u, i = _OPS[r]
            val = res.pop(r)
            if kind == "qk":
                last = u
                exponentiate(u, i, val)
            elif u < 0:
                val = jnp.concatenate(
                    [handoff[zl + (_A_LAST + 10 + n)] for n in range(2)], axis=0) + val
                owner = jnp.where(hd > 0, hd - 1, _H)
                _normalize(val, handoff[zl + (_A_LAST + 9)], owner, _NB - 1, o_t, den_s)
            else:
                val = acc[u] = acc[u] + val if i else val
                if i == 15:
                    _normalize(val, den[u], hd + u // _NB, u % _NB, o_t, den_s)
                elif u == _NU - 1 and i == 14:
                    handoff[_A_LAST + 10] = val[:8]
                    handoff[_A_LAST + 11] = val[8:]
                else:
                    paced[zs + (_A_PACE + 3), :, _lanes(3)] = val[8:, _lanes(3)]
        if last is not None and s < end:
            paced[zs + _A_PACE, :, _lanes(s % 4)] = den[last][:, _lanes(s % 4)]
            proj[zs + _R_PACE, :, _lanes(0)] = den[last][:, _lanes((s + 2) % 4)]
    assert not res and not prob
    handoff[_A_LAST + 8, :, _lanes(0)] = proj[zl + (_R_V + hd * _NB + _NU - 1), :, _lanes(3)]
    handoff[_A_LAST + 9] = den[_NU - 1]


def _attend_all(proj, bufs, o_t, den_s):
    handoff = bufs[0][0]
    handoff[pl.ds(_A_LAST, 12)] = jnp.ones((12, 8, _NQ), _F32)
    pl.loop(0, _H // 2)(lambda i: _attend_pair(2 * i, proj, bufs, o_t, den_s))
    p = _unpack(jnp.concatenate([handoff[_A_LAST + g] for g in range(8)], axis=0))
    o = jnp.dot(_unpack(handoff[_A_LAST + 8, :, _lanes(0)]), p, preferred_element_type=_F32)
    o = o + jnp.concatenate([handoff[_A_LAST + 10], handoff[_A_LAST + 11]], axis=0)
    _normalize(o, handoff[_A_LAST + 9], _H - 1, _NB - 1, o_t, den_s)


def _attend_shifted(i, proj, o_t):
    hd, b = i // _NB, i % _NB
    lane0 = pl.multiple_of((hd // 8) * 128, 128)
    q = jnp.concatenate([proj[_R_Q + (2 * hd + n) * _NB + b] for n in range(2)], axis=0)
    row = lax.broadcasted_iota(jnp.int32, (128, _NQ), 0)
    q = jnp.where(row // _DH == hd % 8, jnp.concatenate([q] * 8, axis=0), 0.0).astype(_BF)

    def scores(c):
        k = proj[pl.ds(_R_K + 32 * c, 32), :, pl.ds(lane0, 128)].reshape(256, 128)
        return jnp.dot(_unpack(k), q, preferred_element_type=_F32)

    def running_max(c, m):
        return jnp.maximum(m, jnp.max(scores(c), axis=0, keepdims=True))

    m = lax.fori_loop(0, _NB, running_max, jnp.full((1, _NQ), -jnp.inf, _F32))

    def accumulate(c, sums):
        e = _swap_halves(jnp.exp2(scores(c) - m))
        v = _unpack(proj[_R_V + hd * _NB + c])
        return (sums[0] + jnp.sum(e, axis=0, keepdims=True),
                sums[1] + jnp.dot(v, e.astype(_BF), preferred_element_type=_F32))

    total, o = lax.fori_loop(0, _NB, accumulate,
                             (jnp.zeros((1, _NQ), _F32), jnp.zeros((_DH, _NQ), _F32)))
    o_t[b, pl.ds(pl.multiple_of(hd * 8, 8), 8), :] = _pack((o / total).astype(_BF))


def _kernel(x_hbm, wqkv_hbm, wo_hbm, wr_hbm, wg_hbm, wu_hbm, wd_hbm, out_hbm,
            x_v, wqkv_v, wo_v, wr_v, wg_v, wu_v, wd_v, wq_t, wv_t, first, proj, o_t,
            den_s, ln_s, base_s, out_v, fix_v, in_sem, out_sem, *staging):
    bufs = (staging[:_NBUF], staging[_NBUF:])
    parts = ((0, 256), (256, 256), (512, 512), (1024, 1024))
    x_cp = [pltpu.make_async_copy(x_hbm.at[0, pl.ds(*p)], x_v.at[pl.ds(*p)], in_sem.at[i])
            for i, p in enumerate(parts)]
    wq_cp, wk_cp, wv_cp = [
        pltpu.make_async_copy(wqkv_hbm.at[:, pl.ds(j * _D, _D)], wqkv_v.at[:, pl.ds(j * _D, _D)],
                              in_sem.at[4 + j]) for j in range(3)]
    late_cp = [pltpu.make_async_copy(s, d, in_sem.at[7 + j]) for j, (s, d) in enumerate(
        ((wo_hbm, wo_v), (wr_hbm, wr_v), (wg_hbm, wg_v), (wu_hbm, wu_v), (wd_hbm, wd_v)))]
    for c in (x_cp[0], wk_cp, x_cp[1], x_cp[2], wv_cp, wq_cp, x_cp[3]):
        c.start()

    ln, k_vpu = {}, [jnp.zeros((16, _D), _F32)] * (8 * _KT)

    def norm(lo, n):
        v = _pack(_layernorm(x_v[pl.ds(128 * lo, 128 * n), :].astype(_F32)).astype(_BF))
        ln.update({lo + i: v[64 * i:64 * (i + 1)] for i in range(n)})

    def ln_rows(lo, n):
        return _unpack(jnp.concatenate([ln[i] for i in range(lo, lo + n)], axis=0))

    def project_k(lo, n):
        k = jnp.dot(ln_rows(lo, n), wqkv_v[:, _D:2 * _D], preferred_element_type=_F32)
        k = _swap_halves(k)
        proj[pl.ds(_R_K + 8 * lo, 8 * n)] = _pack(k.astype(_BF)).reshape(8 * n, 8, _D)
        for v, g in enumerate(_VPU_GROUPS):
            if 0 <= g - 8 * lo < 8 * n:
                k_vpu[v] = k[16 * (g - 8 * lo):16 * (g - 8 * lo + 1)]

    def project_v(b, peak):
        v = lax.dot_general(_unpack(wv_t[...]), ln_rows(4 * b, 4), _NT,
                            preferred_element_type=_F32)
        peak = jnp.maximum(peak, jnp.max(jnp.abs(v).reshape(_D // 8, 8, _NQ), axis=0))
        v = _pack(v.astype(_BF))
        for hd in range(_H):
            proj[_R_V + hd * _NB + b] = v[8 * hd:8 * hd + 8]
        return peak

    def project_q(b, hd0, n):
        q = lax.dot_general(_unpack(wq_t[8 * hd0:8 * (hd0 + n)]), ln_rows(4 * b, 4), _NT,
                            preferred_element_type=_F32) * (_DH ** -0.5 * math.log2(math.e))
        packed = _pack(q.astype(_BF))
        for i in range(2 * n):
            proj[_R_Q + (2 * hd0 + i) * _NB + b] = q[8 * i:8 * i + 8]
        for i in range(n):
            proj[_R_QP + (hd0 + i) * _NB + b] = packed[8 * i:8 * i + 8]

    x_cp[0].wait()
    norm(0, 2)
    first[...] = jnp.concatenate([ln[0], ln[1]], axis=0)
    wk_cp.wait()
    ln[0], ln[1] = first[:64], first[64:]
    project_k(0, 1)
    x_cp[1].wait()
    project_k(1, 1)
    norm(2, 2)
    project_k(2, 1)
    x_cp[2].wait()
    project_k(3, 1)
    norm(4, 4)
    project_k(4, 2)
    wv_cp.wait()
    wq_cp.wait()
    project_k(6, 2)
    wv_t[...] = _pack(wqkv_v[:, 2 * _D:].T)
    v_peak = project_v(0, jnp.zeros((8, _NQ), _F32))
    x_cp[3].wait()
    for c in late_cp:
        c.start()
    v_peak = project_v(1, v_peak)
    norm(8, 4)
    project_k(8, 4)
    norm(12, 4)
    wq_t[...] = _pack(wqkv_v[:, :_D].T)
    project_k(12, 4)
    proj[pl.ds(_R_KT, 2 * _H), :, :128 * _KT] = jnp.concatenate(k_vpu, axis=0).T.reshape(
        2 * _H, 8, 128 * _KT)
    for b in (2, 3):
        v_peak = project_v(b, v_peak)
    for b in range(_NB):
        project_q(b, 0, 8)
    for _, job, args in _staging_jobs(proj, bufs[0], 0, 0):
        job(*args)
    for b in range(_NB):
        project_q(b, 8, _H - 8)
    for c in late_cp:
        c.wait()

    def o_rows(lo):
        return _pack(_unpack(o_t[lo // _NQ, :_D // 2, lo % _NQ:lo % _NQ + 128]).T)

    _attend_all(proj, bufs, o_t, den_s)
    den = den_s[:_H * _NB]
    safe = jnp.where(den > 2.0 ** -30, jnp.where(den < 2.0 ** 60, 1.0, 0.0), 0.0)
    safe = jnp.where(v_peak < 2.0 ** 60, jnp.min(safe.reshape(-1, 8, _NQ), axis=0), 0.0)
    first[:64] = o_rows(0)

    @pl.when(jnp.min(safe) < 0.5)
    def _():
        pl.loop(0, _H * _NB)(lambda i: _attend_shifted(i, proj, o_t))
        first[:64] = o_rows(0)

    parts = ((0, 1024), (1024, 512), (1536, 512))
    out_cp = [pltpu.make_async_copy(out_v.at[pl.ds(*p)], out_hbm.at[0, pl.ds(*p)], out_sem.at[i])
              for i, p in enumerate(parts)]
    wr = wr_v[...].astype(_F32).reshape(1, _D)
    v1 = v2 = jnp.full((8, 1), -jnp.inf, _F32)
    g1, g2 = jnp.zeros((8, 1), jnp.int32), jnp.ones((8, 1), jnp.int32)
    for lo in range(0, _S, 128):
        o = o_rows(lo) if lo else first[:64]
        attn = jnp.dot(_unpack(o), wo_v[...], preferred_element_type=_F32)
        for c, p in zip(out_cp, parts):
            if lo == sum(p) + 128:
                c.start()
        h = x_v[lo:lo + 128, :].astype(_F32) + attn
        cen = h - jnp.mean(h, axis=-1, keepdims=True)
        rstd = lax.rsqrt(jnp.mean(cen * cen, axis=-1, keepdims=True) + _EPS)
        score = jnp.sum(cen * wr, axis=-1, keepdims=True) * rstd
        ln2 = cen * rstd
        base = h + ln2
        ln_s[lo:lo + 128, :] = ln2
        base_s[lo:lo + 128, :] = base
        out_v[lo:lo + 128, :] = base.astype(_BF)
        for i in range(16):
            r, g = score[8 * i:8 * i + 8], lo // 8 + i
            new1, new2 = r > v1, r > v2
            v2 = jnp.where(new1, v1, jnp.where(new2, r, v2))
            g2 = jnp.where(new1, g1, jnp.where(new2, g, g2))
            v1 = jnp.where(new1, r, v1)
            g1 = jnp.where(new1, g, g1)
    out_cp[2].start()

    def best(v, token):
        m = jnp.max(v, axis=0, keepdims=True)
        return m, jnp.min(jnp.where(v == m, token, _S), axis=0, keepdims=True)

    sub = lax.broadcasted_iota(jnp.int32, (8, 1), 0)
    m1, i1 = best(v1, 8 * g1 + sub)
    taken = 8 * g1 + sub == i1
    m2, i2 = best(jnp.where(taken, v2, v1), 8 * jnp.where(taken, g2, g1) + sub)
    t1, t2 = i1[0, 0] & (_S - 1), i2[0, 0] & (_S - 1)
    groups = [pl.multiple_of(t & (_S - 16), 16) for t in (t1, t2)]
    xs = jnp.concatenate([ln_s[pl.ds(g, 16), :] for g in groups], axis=0).astype(_BF)
    gate = jnp.dot(xs, wg_v[...], preferred_element_type=_F32)
    up = jnp.dot(xs, wu_v[...], preferred_element_type=_F32)
    act = (gate * jax.nn.sigmoid(gate) * up).astype(_BF)
    y = jnp.dot(act, wd_v[...], preferred_element_type=_F32)
    y1, y2 = y[:16] * jax.nn.sigmoid(m1), y[16:] * jax.nn.sigmoid(m2)
    row = lax.broadcasted_iota(jnp.int32, (16, _D), 0)
    for i, g in enumerate(groups):
        update = jnp.where(row == t1 - g, y1, jnp.where(row == t2 - g, y2, 0.0))
        fix_v[i] = (base_s[pl.ds(g, 16), :] + update).astype(_BF)
    for c in out_cp:
        c.wait()
    fix_cp = [pltpu.make_async_copy(fix_v.at[i], out_hbm.at[0, pl.ds(g, 16)], out_sem.at[i])
              for i, g in enumerate(groups)]
    fix_cp[0].start()

    @pl.when(groups[0] != groups[1])
    def _():
        fix_cp[1].start()
        fix_cp[1].wait()

    fix_cp[0].wait()


@jax.jit
def pallas_sequential_preLN__mha_block__moe_arch_mod__prompt_kernel(
    A_x: jax.Array,
    A_wqkv: jax.Array,
    A_wo: jax.Array,
    B_x: jax.Array,
    B_w_r: jax.Array,
    B_w_gate: jax.Array,
    B_w_up: jax.Array,
    B_w_down: jax.Array,
):
    del B_x
    assert A_x.shape == (1, _S, _D)
    inputs = (A_x, A_wqkv, A_wo, B_w_r, B_w_gate, B_w_up, B_w_down)
    in_hbm = pl.BlockSpec(memory_space=pl.ANY)
    return pl.pallas_call(
        _kernel,
        out_shape=jax.ShapeDtypeStruct(A_x.shape, A_x.dtype),
        in_specs=[in_hbm] * len(inputs),
        out_specs=in_hbm,
        scratch_shapes=[pltpu.VMEM((_S, _D), _BF)]
        + [pltpu.VMEM(w.shape, _BF) for w in inputs[1:]]
        + [
            pltpu.VMEM((_D // 2, _D), _F32),
            pltpu.VMEM((_D // 2, _D), _F32),
            pltpu.VMEM((128, _D), _F32),
            pltpu.VMEM((_R_ROWS, 8, _NQ), _F32),
            pltpu.VMEM((_NB, _D // 2 + 8, _NQ), _F32),
            pltpu.VMEM(((_H + 2) * _NB, _NQ), _F32),
            pltpu.VMEM((_S, _D), _F32),
            pltpu.VMEM((_S, _D), _F32),
            pltpu.VMEM((_S, _D), _BF),
            pltpu.VMEM((2, 16, _D), _BF),
            pltpu.SemaphoreType.DMA((12,)),
            pltpu.SemaphoreType.DMA((3,)),
        ]
        + [pltpu.VMEM((_A_ROWS, 8, _NQ), _F32)] * (2 * _NBUF),
        compiler_params=pltpu.CompilerParams(vmem_limit_bytes=100 * 2 ** 20),
        name="fused_block",
    )(*inputs)
```
